```python
import os as _os
_os.environ.setdefault("JAX_PLATFORMS", "cpu")
import jax
import jax.numpy as jnp

def _softmax(x, axis=-1):
    return jax.nn.softmax(x, axis=axis)
def _gelu(x):
    return jax.nn.gelu(x, approximate=True)
def _silu(x):
    return jax.nn.silu(x)
def _sigmoid(x):
    return jax.nn.sigmoid(x)
def _layernorm(x, axis=-1, eps=1e-5):
    m = jnp.mean(x, axis=axis, keepdims=True)
    v = jnp.var(x, axis=axis, keepdims=True)
    return (x - m) / jnp.sqrt(v + eps)
def _scatter_add(tgt, idx, src, axis=0):
    return tgt.at[idx].add(src)
def _segment_sum(src, seg, n):
    return jax.ops.segment_sum(src, seg, n)
class _Rng:
    def __init__(self, key):
        self._k = key
    def _next(self):
        self._k, sub = jax.random.split(self._k)
        return sub
    def normal(self, shape):
        return jax.random.normal(self._next(), shape, dtype=jnp.bfloat16)
    def randint(self, lo, hi, shape):
        return jax.random.randint(self._next(), shape, lo, hi, dtype=jnp.int32)
    def uniform(self, shape, lo=0.0, hi=1.0):
        return jax.random.uniform(self._next(), shape, jnp.bfloat16, lo, hi)
    def permutation(self, n):
        return jax.random.permutation(self._next(), n)


kernel_name = 'sequential_preLN__mha_block__moe_arch_mod__prompt'

def setup_inputs():
    _rng = _Rng(jax.random.key(int.from_bytes(__import__("os").urandom(4), "little")))
    _w = (lambda a: (lambda t: t.astype(jnp.bfloat16) if jnp.issubdtype(t.dtype, jnp.floating) else t)(jnp.asarray(a)))
    def _A_setup():
        B, S, D, H = 1, 2048, 640, 32
        return {
            "x": _w((lambda *s: _rng.normal(s) * 0.05)(B, S, D)),
            "wqkv": _w((lambda *s: _rng.normal(s) * 0.05)(D, 3 * D)),
            "wo": _w((lambda *s: _rng.normal(s) * 0.05)(D, D)),
        }
    _A_in = _A_setup()

    def _B_setup():
        B, S, D, F, C = 1, 2048, 640, 1536, 1
        return {
            "x": _w((lambda *s: _rng.normal(s) * 0.05)(B, S, D)),
            "w_r": _w((lambda *s: _rng.normal(s) * 0.05)(D)),
            "w_gate": _w((lambda *s: _rng.normal(s) * 0.05)(D, F)),
            "w_up": _w((lambda *s: _rng.normal(s) * 0.05)(D, F)),
            "w_down": _w((lambda *s: _rng.normal(s) * 0.05)(F, D)),
        }
    _B_in = _B_setup()

    return {
        "A_x": _A_in["x"],
        "A_wqkv": _A_in["wqkv"],
        "A_wo": _A_in["wo"],
        "B_x": _B_in["x"],
        "B_w_r": _B_in["w_r"],
        "B_w_gate": _B_in["w_gate"],
        "B_w_up": _B_in["w_up"],
        "B_w_down": _B_in["w_down"],
    }

def reference(A_x, A_wqkv, A_wo, B_x, B_w_r, B_w_gate, B_w_up, B_w_down):
    def _A_ref(x, wqkv, wo):
        B, S, D = x.shape
        H = 32
        Dh = D // H
        qkv = (lambda x, *d: x.transpose(*d))((x @ wqkv).reshape(B, S, 3, H, Dh), 2, 0, 3, 1, 4)
        q, k, v = qkv[0], qkv[1], qkv[2]
        scores = jnp.einsum("bhqd,bhkd->bhqk", q, k) * (Dh ** -0.5)
        p = _softmax(scores, axis=-1)
        o = jnp.einsum("bhqk,bhkd->bhqd", p, v)
        return (lambda x, *d: x.transpose(*d))(o, 0, 2, 1, 3).reshape(B, S, D) @ wo

    def _B_ref(x, w_r, w_gate, w_up, w_down):
        B, S, D = x.shape
        C = 1
        r = x @ w_r
        idx = jnp.argsort(-r, axis=-1)[:, :C]
        idx_e = jnp.repeat(idx.reshape(B, C, 1), D, axis=2)
        x_sel = jnp.take_along_axis(x, idx_e, axis=1)
        g = _silu(x_sel @ w_gate)
        u = x_sel @ w_up
        y = (g * u) @ w_down
        r_sel = _sigmoid(jnp.take_along_axis(r, idx, axis=1))
        y = y * r_sel.reshape(B, C, 1)
        b_off = (jnp.arange(B) * S).reshape(B, 1)
        flat_idx = (idx + b_off).reshape(B * C)
        zero = (x * 0.0).reshape(B * S, D)
        upd = _scatter_add(zero, flat_idx, y.reshape(B * C, D), axis=0)
        return x + upd.reshape(B, S, D)

    x = A_x
    h = x + _A_ref(_layernorm(x, axis=-1), A_wqkv, A_wo)
    h2 = h + _B_ref(_layernorm(h, axis=-1), B_w_r, B_w_gate, B_w_up, B_w_down)
    return h2
```

```python
import functools
import math
import numpy as np
import jax
import jax.numpy as jnp
from jax import lax
import jax.experimental.pallas as pl
import jax.experimental.pallas.tpu as pltpu

S = 2048
D = 640
H = 32
DH = 20
F = 1536
NG = 6
BQ = 512
BK = 128
NQB = S // BQ
NKB = S // BK
EPS = 1e-5
QSCALE = (DH ** -0.5) * math.log2(math.e)

f32 = jnp.float32
bf16 = jnp.bfloat16
u32 = jnp.uint32


def make_kernel(nsteps=4, TCH=256, ECH=256, dbg=None):
    NUNITS = H * NQB

    def kernel(x_hbm, wqkv_hbm, wo_hbm, wr_hbm, wg_hbm, wu_hbm, wd_hbm, out_hbm,
               x_v, wqkv_v, wo_v, wr_v, wg_v, wu_v, wd_v,
               wqT_v, wvT_v, xn_v, k_v, qt_v, vt_v, sa_v, sb_v, ot_v, h_v, o_v, patch_v,
               z_s, sems, osems):
        cp_w = pltpu.make_async_copy(wqkv_hbm, wqkv_v, sems.at[0])
        cp_x = pltpu.make_async_copy(x_hbm, x_v, sems.at[1])
        cp_wo = pltpu.make_async_copy(wo_hbm, wo_v, sems.at[2])
        cp_wr = pltpu.make_async_copy(wr_hbm, wr_v, sems.at[3])
        cp_wg = pltpu.make_async_copy(wg_hbm, wg_v, sems.at[4])
        cp_wu = pltpu.make_async_copy(wu_hbm, wu_v, sems.at[5])
        cp_wd = pltpu.make_async_copy(wd_hbm, wd_v, sems.at[6])
        cp_w.start()
        cp_x.start()
        z_s[0] = 0

        cp_w.wait()
        wqT_v[...] = wqkv_v[:, 0:D].astype(f32).T.astype(bf16)
        wvT_v[...] = wqkv_v[:, 2 * D:3 * D].astype(f32).T.astype(bf16)
        cp_x.wait()
        cp_wo.start(); cp_wr.start(); cp_wg.start(); cp_wu.start(); cp_wd.start()

        def layernorm(xf):
            m = jnp.mean(xf, axis=-1, keepdims=True)
            c = xf - m
            v = jnp.mean(c * c, axis=-1, keepdims=True)
            return c * lax.rsqrt(v + EPS)

        def proj_chunk(c, carry):
            ts = pl.ds(pl.multiple_of(c * TCH, TCH), TCH)
            xn = layernorm(x_v[ts, :].astype(f32)).astype(bf16)
            k = jnp.dot(xn, wqkv_v[:, D:2 * D], preferred_element_type=f32).astype(bf16)
            ku = pltpu.bitcast(k, u32)
            ts2 = pl.ds(pl.multiple_of(c * (TCH // 2), TCH // 2), TCH // 2)
            for g in range(NG - 1):
                k_v[ts2, g * 128:(g + 1) * 128] = ku[:, 120 * g:120 * g + 128]
            k_v[ts2, 5 * 128:6 * 128] = jnp.concatenate(
                [ku[:, 600:640], jnp.zeros((TCH // 2, 88), u32)], axis=1)
            nt = (((1,), (1,)), ((), ()))
            qt = lax.dot_general(wqT_v[...], xn, nt, preferred_element_type=f32) * QSCALE
            for g in range(NG - 1):
                qt_v[g * 64:(g + 1) * 64, ts] = pltpu.bitcast(qt[120 * g:120 * g + 128, :].astype(bf16), u32)
            qlast = jnp.concatenate([qt[600:640, :], jnp.zeros((88, TCH), f32)], axis=0)
            qt_v[5 * 64:6 * 64, ts] = pltpu.bitcast(qlast.astype(bf16), u32)
            vt = lax.dot_general(wvT_v[...], xn, nt, preferred_element_type=f32)
            vt = vt.astype(bf16).astype(f32)
            row = lax.broadcasted_iota(jnp.int32, (4, TCH), 0)
            ones4 = jnp.where(row == 0, 1.0, 0.0).astype(f32)
            for h in range(H):
                vt_v[24 * h:24 * h + 24, ts] = jnp.concatenate([vt[20 * h:20 * h + 20, :], ones4], axis=0)
            return carry

        lax.fori_loop(0, S // TCH, proj_chunk, 0)

        def get_qt(h, qb):
            g = h // 6
            j = h - g * 6
            qt = qt_v[pl.ds(pl.multiple_of(g * 64, 64), 64), pl.ds(pl.multiple_of(qb * BQ, BQ), BQ)]
            rows = lax.broadcasted_iota(jnp.int32, (64, BQ), 0)
            qt = jnp.where((rows >= j * 10) & (rows < j * 10 + 10), qt, jnp.zeros_like(qt))
            return g, pltpu.bitcast(qt, bf16)

        def ldk(kb, g):
            kk = k_v[pl.ds(kb * (BK // 2), BK // 2), pl.ds(pl.multiple_of(g * 128, 128), 128)]
            return pltpu.bitcast(kk, bf16)

        def step(u, m_cur, s_cur, s_nxt, zoff):
            un = jnp.minimum(u + 1, NUNITS - 1)
            g, qt = get_qt(un // NQB, un % NQB)
            h = u // NQB
            qb = u % NQB
            m_n = jnp.full((8, BQ), -jnp.inf, f32)
            acc = jnp.zeros((24, BQ), f32)
            for kb in range(NKB):
                ks = pl.ds(kb * BK, BK)
                st = jnp.dot(ldk(kb, g), qt, preferred_element_type=f32)
                s_nxt[ks, :] = st
                m_n = jnp.maximum(m_n, jnp.max(st.reshape(BK // 8, 8, BQ), axis=0))
                kso = pl.ds(pl.multiple_of(zoff + kb * BK, 8), BK)
                p = jnp.exp2(s_cur[kso, :] - m_cur).astype(bf16)
                vt = vt_v[pl.ds(pl.multiple_of(h * 24, 8), 24), ks]
                acc = acc + jnp.dot(vt, p, preferred_element_type=f32)
            o = acc * (1.0 / acc[20:21])
            ot_v[pl.ds(pl.multiple_of(h * 24, 8), 24), pl.ds(pl.multiple_of(qb * BQ, BQ), BQ)] = o
            return jnp.max(m_n, axis=0, keepdims=True)

        def body(i, m):
            zoff = z_s[0]
            bufs = [sa_v, sb_v]
            for s in range(nsteps):
                m = step(nsteps * i + s, m, bufs[s % 2], bufs[(s + 1) % 2], zoff)
            return m

        g0, qt0 = get_qt(0, 0)
        m_n = jnp.full((8, BQ), -jnp.inf, f32)
        for kb in range(NKB):
            ks = pl.ds(kb * BK, BK)
            st = jnp.dot(ldk(kb, 0), qt0, preferred_element_type=f32)
            sa_v[ks, :] = st
            m_n = jnp.maximum(m_n, jnp.max(st.reshape(BK // 8, 8, BQ), axis=0))
        m0 = jnp.max(m_n, axis=0, keepdims=True)
        lax.fori_loop(0, NUNITS // nsteps, body, m0)

        cp_wo.wait(); cp_wr.wait()
        wo_f = wo_v[...].astype(f32)
        z4 = jnp.zeros((4, D), f32)
        wo_pad = jnp.concatenate(
            [jnp.concatenate([wo_f[20 * h:20 * h + 20, :], z4], axis=0) for h in range(H)], axis=0).astype(bf16)
        wr = wr_v[...].astype(f32).reshape(1, D)
        NE = S // ECH

        def out_copy(c):
            ts = pl.ds(pl.multiple_of(c * ECH, ECH), ECH)
            return pltpu.make_async_copy(o_v.at[ts, :], out_hbm.at[ts, :], osems.at[c])

        def epi_chunk(c, carry):
            best, bidx = carry
            ts = pl.ds(pl.multiple_of(c * ECH, ECH), ECH)
            ot = ot_v[:, ts]
            o = ot.T.astype(bf16)
            attn = jnp.dot(o, wo_pad, preferred_element_type=f32)
            hh = x_v[ts, :].astype(f32) + attn
            x2 = layernorm(hh)
            r = jnp.sum(x2.astype(bf16).astype(f32) * wr, axis=-1, keepdims=True)
            r = r.astype(bf16).astype(f32)
            h_v[ts, :] = hh
            o_v[ts, :] = (hh + x2).astype(bf16)
            out_copy(c).start()
            rid = lax.broadcasted_iota(jnp.int32, (ECH, 1), 0) + c * ECH
            take = r > best
            best = jnp.where(take, r, best)
            bidx = jnp.where(take, rid, bidx)
            return best, bidx

        best, bidx = lax.fori_loop(
            0, NE, epi_chunk,
            (jnp.full((ECH, 1), -jnp.inf, f32), jnp.zeros((ECH, 1), jnp.int32)))
        rmax = jnp.max(best, axis=0, keepdims=True)
        cand = jnp.where(best == rmax, bidx, S)
        idx_v = jnp.min(cand.astype(f32), axis=0, keepdims=True)
        idx = jnp.clip(idx_v[0, 0].astype(jnp.int32), 0, S - 1)

        cp_wg.wait(); cp_wu.wait(); cp_wd.wait()
        base = pl.multiple_of((idx // 16) * 16, 16)
        rs = pl.ds(base, 16)
        hh = h_v[rs, :]
        x2 = layernorm(hh)
        x2b = x2.astype(bf16)
        gg = jnp.dot(x2b, wg_v[...], preferred_element_type=f32)
        uu = jnp.dot(x2b, wu_v[...], preferred_element_type=f32)
        act = (gg * jax.nn.sigmoid(gg)) * uu
        y = jnp.dot(act.astype(bf16), wd_v[...], preferred_element_type=f32)
        y = y * jax.nn.sigmoid(rmax)
        sel = lax.broadcasted_iota(jnp.int32, (16, D), 0) == (idx - base)
        res = hh + x2 + jnp.where(sel, y, 0.0)
        patch_v[...] = res.astype(bf16)
        for c in range(NE):
            out_copy(c).wait()
        cp_p = pltpu.make_async_copy(patch_v, out_hbm.at[rs, :], sems.at[7])
        cp_p.start()
        cp_p.wait()

    return kernel


def build(nsteps=4, TCH=256, ECH=256, vmem_mb=100, **kw):
    kernel = make_kernel(nsteps=nsteps, TCH=TCH, ECH=ECH)

    def fn(A_x, A_wqkv, A_wo, B_x, B_w_r, B_w_gate, B_w_up, B_w_down):
        x2d = A_x.reshape(S, D)
        wr = B_w_r
        any_spec = pl.BlockSpec(memory_space=pl.ANY)
        out = pl.pallas_call(
            kernel,
            out_shape=jax.ShapeDtypeStruct((S, D), bf16),
            in_specs=[any_spec] * 7,
            out_specs=any_spec,
            scratch_shapes=[
                pltpu.VMEM((S, D), bf16),
                pltpu.VMEM((D, 3 * D), bf16),
                pltpu.VMEM((D, D), bf16),
                pltpu.VMEM((D,), bf16),
                pltpu.VMEM((D, F), bf16),
                pltpu.VMEM((D, F), bf16),
                pltpu.VMEM((F, D), bf16),
                pltpu.VMEM((D, D), bf16),
                pltpu.VMEM((D, D), bf16),
                pltpu.VMEM((S, D), bf16),
                pltpu.VMEM((S // 2, NG * 128), u32),
                pltpu.VMEM((NG * 64, S), u32),
                pltpu.VMEM((H * 24, S), f32),
                pltpu.VMEM((S, BQ), f32),
                pltpu.VMEM((S, BQ), f32),
                pltpu.VMEM((H * 24, S), f32),
                pltpu.VMEM((S, D), f32),
                pltpu.VMEM((S, D), bf16),
                pltpu.VMEM((16, D), bf16),
                pltpu.SMEM((1,), jnp.int32),
                pltpu.SemaphoreType.DMA((8,)),
                pltpu.SemaphoreType.DMA((S // ECH,)),
            ],
            compiler_params=pltpu.CompilerParams(vmem_limit_bytes=vmem_mb * 1024 * 1024),
        )(x2d, A_wqkv, A_wo, wr, B_w_gate, B_w_up, B_w_down)
        return out.reshape(1, S, D)

    return jax.jit(fn)


_impl = build()


@jax.jit
def pallas_sequential_preLN__mha_block__moe_arch_mod__prompt_kernel(
    A_x, A_wqkv, A_wo, B_x, B_w_r, B_w_gate, B_w_up, B_w_down):
    return _impl(A_x, A_wqkv, A_wo, B_x, B_w_r, B_w_gate, B_w_up, B_w_down)
```

```python
import math

import jax
import jax.numpy as jnp
from jax import lax
import jax.experimental.pallas as pl
import jax.experimental.pallas.tpu as pltpu

S = 2048
D = 640
H = 32
DH = 20
F = 1536
EPS = 1e-5

NG = 6
BQ = 512
BK = 128
NQB = S // BQ
NKB = S // BK
VR = 24
NSTEPS = 8
LAG = 2
QSCALE = (DH ** -0.5) * math.log2(math.e)

TCH = 256
NTC = S // TCH
RB = 32
KA = 384
ECH = 128
DCH = 256
NE = S // ECH
ND = S // DCH

f32 = jnp.float32
bf16 = jnp.bfloat16
u32 = jnp.uint32
NT = (((1,), (1,)), ((), ()))
TN = (((0,), (0,)), ((), ()))


def _layernorm(xf):
    m = jnp.mean(xf, axis=-1, keepdims=True)
    c = xf - m
    v = jnp.mean(c * c, axis=-1, keepdims=True)
    return c * lax.rsqrt(v + EPS)


def _kernel(x_hbm, wqkv_hbm, wo_hbm, wr_hbm, wg_hbm, wu_hbm, wd_hbm, out_hbm,
            x_v, wq_v, wk_v, wv_v, wo_v, wr_v, wg_v, wu_v, wd_v,
            wqT_v, wvT_v, xn_v, k_v, knat_v, qt_v, vt_v, sa_v, sb_v, ot_v, x2_v, o_v, patch_v,
            z_s, sems, xsems, osems):
    cp_wka = pltpu.make_async_copy(wqkv_hbm.at[:, D:D + KA], wk_v.at[:, 0:KA], sems.at[0])
    cp_wkb = pltpu.make_async_copy(wqkv_hbm.at[:, D + KA:2 * D], wk_v.at[:, KA:D], sems.at[1])
    cp_wq = pltpu.make_async_copy(wqkv_hbm.at[:, 0:D], wq_v, sems.at[2])
    cp_wv = pltpu.make_async_copy(wqkv_hbm.at[:, 2 * D:3 * D], wv_v, sems.at[3])
    cp_wo = pltpu.make_async_copy(wo_hbm, wo_v, sems.at[4])
    cp_wr = pltpu.make_async_copy(wr_hbm, wr_v, sems.at[5])
    cp_wg = pltpu.make_async_copy(wg_hbm, wg_v, sems.at[6])
    cp_wu = pltpu.make_async_copy(wu_hbm, wu_v, sems.at[7])
    cp_wd = pltpu.make_async_copy(wd_hbm, wd_v, sems.at[8])

    def cp_x(c):
        ts = pl.ds(c * TCH, TCH)
        return pltpu.make_async_copy(x_hbm.at[ts, :], x_v.at[ts, :], xsems.at[c])

    def cp_out(c):
        ts = pl.ds(c * DCH, DCH)
        return pltpu.make_async_copy(o_v.at[ts, :], out_hbm.at[ts, :], osems.at[c])

    cp_x(0).start()
    cp_wka.start()
    cp_wkb.start()
    z_s[0] = 0
    sa_v[...] = jnp.zeros((S, BQ), f32)

    def ln1(c):
        for r in range(TCH // RB):
            ts = pl.ds(c * TCH + r * RB, RB)
            xn_v[ts, :] = _layernorm(x_v[ts, :].astype(f32)).astype(bf16)

    def k_relayout(c, ku):
        ts = pl.ds(c * (TCH // 2), TCH // 2)
        for g in range(NG - 1):
            k_v[ts, g * 128:(g + 1) * 128] = ku[:, 120 * g:120 * g + 128]
        k_v[ts, 5 * 128:6 * 128] = jnp.concatenate(
            [ku[:, 600:640], jnp.zeros((TCH // 2, 88), u32)], axis=1)

    def kproj(c):
        xn = xn_v[pl.ds(c * TCH, TCH), :]
        k = jnp.dot(xn, wk_v[...], preferred_element_type=f32).astype(bf16)
        k_relayout(c, pltpu.bitcast(k, u32))

    cp_x(0).wait()
    cp_x(1).start(); cp_x(2).start()
    ln1(0)
    cp_wka.wait()
    ka = jnp.dot(xn_v[0:TCH, :], wk_v[:, 0:KA], preferred_element_type=f32).astype(bf16)
    knat_v[:, 0:KA] = pltpu.bitcast(ka, u32)
    cp_wkb.wait(); cp_x(1).wait()
    cp_x(3).start(); cp_x(4).start(); cp_x(5).start()
    kb_ = jnp.dot(xn_v[0:TCH, :], wk_v[:, KA:D], preferred_element_type=f32).astype(bf16)
    ln1(1)
    k_relayout(0, jnp.concatenate([knat_v[:, 0:KA], pltpu.bitcast(kb_, u32)], axis=1))
    cp_x(2).wait()
    cp_x(6).start(); cp_x(7).start(); cp_wq.start(); cp_wv.start()
    kproj(1); ln1(2)
    cp_x(3).wait(); cp_x(4).wait(); cp_x(5).wait()
    kproj(2); ln1(3); kproj(3); ln1(4); kproj(4); ln1(5)
    cp_x(6).wait(); cp_x(7).wait(); cp_wq.wait(); cp_wv.wait()
    cp_wo.start(); cp_wr.start(); cp_wg.start(); cp_wu.start(); cp_wd.start()
    kproj(5); ln1(6)
    wqT_v[...] = wq_v[...].astype(f32).T.astype(bf16)
    wvT_v[...] = wv_v[...].astype(f32).T.astype(bf16)
    kproj(6); ln1(7); kproj(7)

    for c in range(NTC):
        ts = pl.ds(c * TCH, TCH)
        xn = xn_v[ts, :]
        qt = lax.dot_general(wqT_v[...], xn, NT, preferred_element_type=f32) * QSCALE
        for g in range(NG - 1):
            qt_v[g * 64:(g + 1) * 64, ts] = pltpu.bitcast(qt[120 * g:120 * g + 128, :].astype(bf16), u32)
        qlast = jnp.concatenate([qt[600:640, :], jnp.zeros((88, TCH), f32)], axis=0)
        qt_v[5 * 64:6 * 64, ts] = pltpu.bitcast(qlast.astype(bf16), u32)
        vt = lax.dot_general(wvT_v[...], xn, NT, preferred_element_type=f32)
        row = lax.broadcasted_iota(jnp.int32, (VR - DH, TCH), 0)
        ones4 = jnp.where(row == 0, 1.0, 0.0).astype(f32)
        for h in range(H):
            vt_v[VR * h:VR * (h + 1), ts] = jnp.concatenate([vt[DH * h:DH * (h + 1), :], ones4], axis=0)

    def get_qt(h, qb):
        g = h // 6
        j = h - g * 6
        qt = qt_v[pl.ds(pl.multiple_of(g * 64, 64), 64), pl.ds(qb * BQ, BQ)]
        rows = lax.broadcasted_iota(jnp.int32, (64, BQ), 0)
        qt = jnp.where((rows >= j * 10) & (rows < j * 10 + 10), qt, jnp.zeros_like(qt))
        return g, pltpu.bitcast(qt, bf16)

    def load_k(kb, g):
        kk = k_v[pl.ds(kb * (BK // 2), BK // 2), pl.ds(pl.multiple_of(g * 128, 128), 128)]
        return pltpu.bitcast(kk, bf16)

    def pv_dot(kb, h, m_cur, s_cur, zoff):
        ks = pl.ds(kb * BK, BK)
        kso = pl.ds(pl.multiple_of(zoff + kb * BK, 8), BK)
        p = jnp.exp2(s_cur[kso, :] - m_cur).astype(bf16)
        vt = vt_v[pl.ds(pl.multiple_of(h * VR, 8), VR), ks]
        return jnp.dot(vt, p, preferred_element_type=f32)

    def pv_store(acc, h, qb, hpar):
        o = acc[0:DH] * (1.0 / acc[DH:DH + 1])
        qs = pl.ds(qb * BQ, BQ)
        if hpar == 0:
            ot_v.at[pl.ds(pl.multiple_of(h * DH, 8), 2 * DH), qs][0:DH, :] = o
        else:
            ot_v.at[pl.ds(pl.multiple_of((h - 1) * DH, 8), 2 * DH), qs][DH:2 * DH, :] = o

    def step(h, qb, hn, qbn, m_cur, s_cur, s_nxt, zoff, hpar):
        g, qt = get_qt(hn, qbn)
        m_n = jnp.full((8, BQ), -jnp.inf, f32)
        acc = jnp.zeros((VR, BQ), f32)
        for n in range(NKB + LAG):
            if n < NKB:
                st = jnp.dot(load_k(n, g), qt, preferred_element_type=f32)
                s_nxt[pl.ds(n * BK, BK), :] = st
                m_n = jnp.maximum(m_n, jnp.max(st.reshape(BK // 8, 8, BQ), axis=0))
            if n - LAG >= 0:
                acc = acc + pv_dot(n - LAG, h, m_cur, s_cur, zoff)
        pv_store(acc, h, qb, hpar)
        return jnp.max(m_n, axis=0, keepdims=True)

    HPB = NSTEPS // NQB

    def block(i, m):
        zoff = z_s[0]
        bufs = (sa_v, sb_v)
        for s in range(NSTEPS):
            hn, qbn = i * HPB + s // NQB, s % NQB
            if s == 0:
                h, qb, hpar = jnp.maximum(i * HPB - 1, 1), NQB - 1, 1
            else:
                h, qb, hpar = i * HPB + (s - 1) // NQB, (s - 1) % NQB, ((s - 1) // NQB) % 2
            m = step(h, qb, hn, qbn, m, bufs[s % 2], bufs[(s + 1) % 2], zoff, hpar)
        return m

    m_last = lax.fori_loop(0, H * NQB // NSTEPS, block, jnp.zeros((1, BQ), f32))

    cp_wo.wait()
    cp_wr.wait()
    wr = wr_v[...].astype(f32).reshape(1, D)

    def epi_chunk(c, carry):
        best, bidx = carry
        ts = pl.ds(c * ECH, ECH)
        attn = lax.dot_general(ot_v[:, ts].astype(bf16), wo_v[...], TN, preferred_element_type=f32)
        hh = x_v[ts, :].astype(f32) + attn
        cc = hh - jnp.mean(hh, axis=-1, keepdims=True)
        rstd = lax.rsqrt(jnp.mean(cc * cc, axis=-1, keepdims=True) + EPS)
        score = jnp.sum(cc * wr, axis=-1, keepdims=True)
        x2 = cc * rstd
        r = (score * rstd).astype(bf16).astype(f32)
        x2_v[ts, :] = x2.astype(bf16)
        o_v[ts, :] = (hh + x2).astype(bf16)
        rid = lax.broadcasted_iota(jnp.int32, (ECH, 1), 0) + c * ECH
        take = r > best
        if ((c + 1) * ECH) % DCH == 0:
            cp_out(((c + 1) * ECH) // DCH - 1).start()
        return jnp.where(take, r, best), jnp.where(take, rid, bidx)

    carry = (jnp.full((ECH, 1), -jnp.inf, f32), jnp.zeros((ECH, 1), jnp.int32))
    zoff = z_s[0]
    acc = jnp.zeros((VR, BQ), f32)
    for c in range(NE):
        if c < 2:
            for kb in range(c * (NKB // 2), (c + 1) * (NKB // 2)):
                acc = acc + pv_dot(kb, H - 1, m_last, sa_v, zoff)
        if c == (NQB - 1) * BQ // ECH:
            pv_store(acc, H - 1, NQB - 1, 1)
        carry = epi_chunk(c, carry)
    best, bidx = carry
    rmax = jnp.max(best, axis=0, keepdims=True)
    cand = jnp.where(best == rmax, bidx, S)
    idx = jnp.min(cand.astype(f32), axis=0, keepdims=True)[0, 0].astype(jnp.int32)
    idx = jnp.clip(idx, 0, S - 1)

    cp_wg.wait()
    cp_wu.wait()
    cp_wd.wait()
    base = pl.multiple_of((idx // 16) * 16, 16)
    rs = pl.ds(base, 16)
    x2b = x2_v[rs, :]
    gg = jnp.dot(x2b, wg_v[...], preferred_element_type=f32)
    uu = jnp.dot(x2b, wu_v[...], preferred_element_type=f32)
    act = (gg * jax.nn.sigmoid(gg)) * uu
    y = jnp.dot(act.astype(bf16), wd_v[...], preferred_element_type=f32) * jax.nn.sigmoid(rmax)
    sel = lax.broadcasted_iota(jnp.int32, (16, D), 0) == (idx - base)
    patch_v[...] = (o_v[rs, :].astype(f32) + jnp.where(sel, y, 0.0)).astype(bf16)
    for c in range(ND):
        cp_out(c).wait()
    cp_patch = pltpu.make_async_copy(patch_v, out_hbm.at[rs, :], sems.at[9])
    cp_patch.start()
    cp_patch.wait()


@jax.jit
def pallas_sequential_preLN__mha_block__moe_arch_mod__prompt_kernel(
    A_x: jax.Array,
    A_wqkv: jax.Array,
    A_wo: jax.Array,
    B_x: jax.Array,
    B_w_r: jax.Array,
    B_w_gate: jax.Array,
    B_w_up: jax.Array,
    B_w_down: jax.Array,
):
    del B_x
    hbm = pl.BlockSpec(memory_space=pl.ANY)
    out = pl.pallas_call(
        _kernel,
        out_shape=jax.ShapeDtypeStruct((S, D), bf16),
        in_specs=[hbm] * 7,
        out_specs=hbm,
        scratch_shapes=[
            pltpu.VMEM((S, D), bf16),
            pltpu.VMEM((D, D), bf16),
            pltpu.VMEM((D, D), bf16),
            pltpu.VMEM((D, D), bf16),
            pltpu.VMEM((D, D), bf16),
            pltpu.VMEM((D,), bf16),
            pltpu.VMEM((D, F), bf16),
            pltpu.VMEM((D, F), bf16),
            pltpu.VMEM((F, D), bf16),
            pltpu.VMEM((D, D), bf16),
            pltpu.VMEM((D, D), bf16),
            pltpu.VMEM((S, D), bf16),
            pltpu.VMEM((S // 2, NG * 128), u32),
            pltpu.VMEM((TCH // 2, D), u32),
            pltpu.VMEM((NG * 64, S), u32),
            pltpu.VMEM((H * VR, S), f32),
            pltpu.VMEM((S, BQ), f32),
            pltpu.VMEM((S, BQ), f32),
            pltpu.VMEM((D, S), f32),
            pltpu.VMEM((S, D), bf16),
            pltpu.VMEM((S, D), bf16),
            pltpu.VMEM((16, D), bf16),
            pltpu.SMEM((1,), jnp.int32),
            pltpu.SemaphoreType.DMA((10,)),
            pltpu.SemaphoreType.DMA((NTC,)),
            pltpu.SemaphoreType.DMA((ND,)),
        ],
        compiler_params=pltpu.CompilerParams(
            vmem_limit_bytes=100 * 1024 * 1024,
            flags={"XLA_TPU_EVENLY_DISTRIBUTE_CRITICAL_NODES": True},
        ),
    )(A_x.reshape(S, D), A_wqkv, A_wo, B_w_r, B_w_gate, B_w_up, B_w_down)
    return out.reshape(1, S, D)
```
